```python
import os as _os
_os.environ.setdefault("JAX_PLATFORMS", "cpu")
import jax
import jax.numpy as jnp

def _softmax(x, axis=-1):
    return jax.nn.softmax(x, axis=axis)
def _gelu(x):
    return jax.nn.gelu(x, approximate=True)
def _silu(x):
    return jax.nn.silu(x)
def _sigmoid(x):
    return jax.nn.sigmoid(x)
def _layernorm(x, axis=-1, eps=1e-5):
    m = jnp.mean(x, axis=axis, keepdims=True)
    v = jnp.var(x, axis=axis, keepdims=True)
    return (x - m) / jnp.sqrt(v + eps)
def _scatter_add(tgt, idx, src, axis=0):
    return tgt.at[idx].add(src)
def _segment_sum(src, seg, n):
    return jax.ops.segment_sum(src, seg, n)
class _Rng:
    def __init__(self, key):
        self._k = key
    def _next(self):
        self._k, sub = jax.random.split(self._k)
        return sub
    def normal(self, shape):
        return jax.random.normal(self._next(), shape, dtype=jnp.bfloat16)
    def randint(self, lo, hi, shape):
        return jax.random.randint(self._next(), shape, lo, hi, dtype=jnp.int32)
    def uniform(self, shape, lo=0.0, hi=1.0):
        return jax.random.uniform(self._next(), shape, jnp.bfloat16, lo, hi)
    def permutation(self, n):
        return jax.random.permutation(self._next(), n)


kernel_name = 'standalone__gqa_block_cached__near_ridge'

def setup_inputs():
    _rng = _Rng(jax.random.key(int.from_bytes(__import__("os").urandom(4), "little")))
    _w = (lambda a: (lambda t: t.astype(jnp.bfloat16) if jnp.issubdtype(t.dtype, jnp.floating) else t)(jnp.asarray(a)))
    B, Sq, D = 8, 96, 448
    Hq, Hkv, Sk, Dh = 16, 8, 2048, 256
    assert Hq % Hkv == 0, (Hq, Hkv)
    return {
        "x": _w((lambda *s: _rng.normal(s) * 0.8)(B, Sq, D)),
        "k_cache": _w((lambda *s: _rng.normal(s) * 0.8)(B, Hkv, Sk, Dh)),
        "v_cache": _w((lambda *s: _rng.normal(s) * 0.05)(B, Hkv, Sk, Dh)),
        "wq": _w((lambda *s: _rng.normal(s) * 0.8)(D, Hq * Dh) * (D ** -0.5)),
        "wo": _w((lambda *s: _rng.normal(s) * 0.05)(Hq * Dh, D) * ((Hq * Dh) ** -0.5)),
    }

def reference(x, k_cache, v_cache, wq, wo):
    B, Sq, D = x.shape
    Hq, Dh = 16, 256
    Hkv = k_cache.shape[1]
    rep = Hq // Hkv
    q = (lambda x, *d: x.transpose(*d))((x @ wq).reshape(B, Sq, Hq, Dh), 0, 2, 1, 3)
    k = jnp.repeat(k_cache, rep, axis=1)
    v = jnp.repeat(v_cache, rep, axis=1)
    scores = jnp.einsum("bhqd,bhkd->bhqk", q, k) * (Dh ** -0.5)
    p = _softmax(scores, axis=-1)
    o = jnp.einsum("bhqk,bhkd->bhqd", p, v)
    return (lambda x, *d: x.transpose(*d))(o, 0, 2, 1, 3).reshape(B, Sq, Hq * Dh) @ wo
```

```python
import functools
import math

import jax
import jax.numpy as jnp
from jax import lax
import jax.experimental.pallas as pl
import jax.experimental.pallas.tpu as pltpu

_B, _SQ, _D = 8, 96, 448
_HQ, _HKV, _SK, _DH = 16, 8, 2048, 256
_NU = _B * _HKV
_M = 2 * _SQ
_NB = 4
_CH = 128
_DC = 64
_KS, _VS = 68, 50
_PV = 16
_WS = 4
_NT = (((1,), (1,)), ((), ()))
_QSCALE = math.log2(math.e) * _DH ** -0.5


def _kernel(x_hbm, wq_hbm, woT_hbm, k_hbm, v_hbm, o_hbm,
            x_v, wq_v, wo_v, k_v, v_v, q_v, s_v, p_v, m_v, acc_v, out_v,
            sem_x, sem_wq, sem_wo, sem_k, sem_v, sem_o):
    B, SQ, D, HKV, SK, DH, NU, M = _B, _SQ, _D, _HKV, _SK, _DH, _NU, _M
    NB, CH, DC, KS, VS, WS = _NB, _CH, _DC, _KS, _VS, _WS
    NC = SK // CH
    ND = SK // DC
    PER = ND // NC
    WR = D // B

    def ub(u):
        return u & (B - 1)

    def uj(u):
        return u >> 3 if isinstance(u, int) else lax.shift_right_logical(u, 3)

    def us(u):
        return u & (NB - 1)

    def when(c, f):
        if isinstance(c, bool):
            if c:
                f()
        else:
            pl.when(c)(f)

    def x_all(b):
        return pltpu.make_async_copy(x_hbm.at[b], x_v.at[b], sem_x.at[b])

    def wq_all(j):
        return pltpu.make_async_copy(wq_hbm.at[:, pl.ds(0, 512)], wq_v.at[j], sem_wq.at[j])

    def wo_all(j):
        return pltpu.make_async_copy(woT_hbm.at[:, pl.ds(0, 512)], wo_v.at[j], sem_wo.at[j])

    def k_all(u):
        return pltpu.make_async_copy(k_hbm.at[ub(u), uj(u)], k_v.at[us(u)], sem_k.at[us(u)])

    def v_all(u):
        return pltpu.make_async_copy(v_hbm.at[ub(u), uj(u)], v_v.at[us(u)], sem_v.at[us(u)])

    def o_copy(b):
        return pltpu.make_async_copy(out_v.at[b], o_hbm.at[b], sem_o.at[b])

    def k_start(u, d, prio=0):
        pltpu.make_async_copy(k_hbm.at[ub(u), uj(u), pl.ds(d * DC, DC)],
                              k_v.at[us(u), pl.ds(d * DC, DC)], sem_k.at[us(u)]).start(priority=prio)

    def v_start(u, d, prio=1):
        pltpu.make_async_copy(v_hbm.at[ub(u), uj(u), pl.ds(d * DC, DC)],
                              v_v.at[us(u), pl.ds(d * DC, DC)], sem_v.at[us(u)]).start(priority=prio)

    def issue_k(u, lo, hi):
        for r in range(lo, hi):
            un = u + r // ND
            when(un < NU, functools.partial(k_start, un, r % ND))

    def issue_v(u, lo, hi):
        for r in range(lo, hi):
            un = u + r // ND
            when(un < NU, functools.partial(v_start, un, r % ND))

    def w_issue(u):
        j = uj(u + WS)
        b = ub(u + WS)

        def go():
            for hbm_, vm_, sem_, prio in ((wq_hbm, wq_v, sem_wq, 0), (woT_hbm, wo_v, sem_wo, 1)):
                r0 = b * WR if isinstance(b, int) else pl.multiple_of(b * WR, 8)
                c0 = (j + 1) * 512 if isinstance(j, int) else pl.multiple_of((j + 1) * 512, 128)
                for o_, n_ in ((0, 32), (32, 24)):
                    pltpu.make_async_copy(hbm_.at[pl.ds(r0 + o_, n_), pl.ds(c0, 512)],
                                          vm_.at[j + 1, pl.ds(r0 + o_, n_)],
                                          sem_.at[j + 1]).start(priority=prio)

        when(j + 1 < HKV, go)

    def qproj(u):
        q = jnp.dot(x_v[ub(u)], wq_v[uj(u)], preferred_element_type=jnp.float32) * _QSCALE
        q_v[0:SQ, :] = q[:, :DH].astype(jnp.bfloat16)
        q_v[SQ:M, :] = q[:, DH:].astype(jnp.bfloat16)

    def fold(a, op):
        r = a[:, 0:128]
        for t in range(1, a.shape[1] // 128):
            r = op(r, a[:, t * 128:(t + 1) * 128])
        return r

    def qk_chunk(q, slot, c, mx):
        sl = slice(c * CH, (c + 1) * CH)
        s = lax.dot_general(q, k_v[slot, sl, :], _NT, preferred_element_type=jnp.float32)
        s_v[:, sl] = s
        f = fold(s, jnp.maximum)
        return f if mx is None else jnp.maximum(mx, f)

    def sm_chunk(mrep, c, lp):
        p = jnp.exp2(s_v[:, c * CH:(c + 1) * CH] - mrep)
        f = fold(p, jnp.add)
        return p.astype(jnp.bfloat16), (f if lp is None else lp + f)

    def set_m(mx):
        m_v[...] = jnp.broadcast_to(jnp.max(mx, axis=1, keepdims=True), (M, 128))

    def get_mrep():
        m = m_v[...]
        return m if CH == 128 else jnp.concatenate([m] * (CH // 128), axis=1)

    def pv_chunk(p, slot, c, o):
        pv = jnp.dot(p, v_v[slot, c * CH:(c + 1) * CH, :], preferred_element_type=jnp.float32)
        return pv if o is None else o + pv

    def finish(u, o, lp, do_qp):
        b = ub(u)
        l = jnp.sum(lp, axis=1, keepdims=True)
        on = o * (1.0 / l)
        if do_qp:
            qproj(u + 2)
        w = wo_v[uj(u)]
        y = lax.dot_general(on[0:SQ].astype(jnp.bfloat16), w[:, :DH], _NT,
                            preferred_element_type=jnp.float32)
        y = y + lax.dot_general(on[SQ:M].astype(jnp.bfloat16), w[:, DH:], _NT,
                                preferred_element_type=jnp.float32)
        a = acc_v[b] + y
        acc_v[b] = a
        out_v[b] = a.astype(jnp.bfloat16)
        when(u >= NU - B, lambda: o_copy(b).start())

    for i in range(3):
        pltpu.make_async_copy(x_hbm.at[0, pl.ds(32 * i, 32)], x_v.at[0, pl.ds(32 * i, 32)],
                              sem_x.at[0]).start(priority=i % 2)
    for i in range(14):
        pltpu.make_async_copy(wq_hbm.at[pl.ds(32 * i, 32), pl.ds(0, 512)],
                              wq_v.at[0, pl.ds(32 * i, 32)], sem_wq.at[0]).start(priority=(i + 1) % 2)
    for d in range(ND):
        k_start(0, d, d % 2)
    for i in range(3):
        pltpu.make_async_copy(x_hbm.at[1, pl.ds(32 * i, 32)], x_v.at[1, pl.ds(32 * i, 32)],
                              sem_x.at[1]).start(priority=i % 2)
    for d in range(ND // 2):
        k_start(1, d, d % 2)
    acc_v[...] = jnp.zeros_like(acc_v)

    x_all(0).wait()
    wq_all(0).wait()
    qproj(0)
    for d in range(ND // 2, ND):
        k_start(1, d, d % 2)
    for d in range(_PV):
        v_start(0, d, d % 2)
    k_all(0).wait()
    mx = None
    q = q_v[...]
    for c in range(NC):
        if c == 1:
            for d in range(_PV, ND):
                v_start(0, d, d % 2)
            for h in range(2):
                pltpu.make_async_copy(woT_hbm.at[pl.ds(h * 224, 224), pl.ds(0, 512)],
                                      wo_v.at[0, pl.ds(h * 224, 224)], sem_wo.at[0]).start(priority=h)
        if c == 3:
            for b in range(2, B):
                x_all(b).start(priority=b % 2)
            for uu in range(-WS, 0):
                w_issue(uu)
        mx = qk_chunk(q, 0, c, mx)
    set_m(mx)
    x_all(1).wait()
    qproj(1)
    for r in range(max(KS - 2 * ND, VS - ND)):
        if 2 * ND + r < KS:
            issue_k(0, 2 * ND + r, 2 * ND + r + 1)
        if ND + r < VS:
            issue_v(0, ND + r, ND + r + 1)
    for b in range(2, B):
        x_all(b).wait()

    def step(u, tail=False):
        k_all(u + 1).wait()
        v_all(u).wait()
        when((ub(u + 2) == 0) & (u + 2 < NU), lambda: wq_all(uj(u + 2)).wait())
        when(ub(u) == 0, lambda: wo_all(uj(u)).wait())
        slot = us(u)
        nslot = us(u + 1)
        mrep = get_mrep()
        q = q_v[...]
        lp = mx = o = None
        for c in range(NC):
            issue_v(u, VS + c * PER, VS + (c + 1) * PER)
            p, lp = sm_chunk(mrep, c, lp)
            mx = qk_chunk(q, nslot, c, mx)
            issue_k(u, KS + c * PER, KS + (c + 1) * PER)
            if c == 1:
                w_issue(u)
            o = pv_chunk(p, slot, c, o)
        set_m(mx)
        lp2 = None
        if tail:
            mrep2 = get_mrep()
            for c in range(NC):
                p, lp2 = sm_chunk(mrep2, c, lp2)
                p_v[:, c * CH:(c + 1) * CH] = p
        finish(u, o, lp, not tail)
        return lp2

    def loop(i, carry):
        step(i)
        return carry

    lax.fori_loop(0, NU - 2, loop, 0)
    lp2 = step(NU - 2, tail=True)
    issue_v(NU - 2, VS + ND, 4 * ND)
    issue_k(NU - 2, KS + ND, 4 * ND)

    u = NU - 1
    v_all(u).wait()
    o = None
    for c in range(NC):
        o = pv_chunk(p_v[:, c * CH:(c + 1) * CH], us(u), c, o)
    finish(u, o, lp2, False)
    for b in range(B):
        o_copy(b).wait()


@jax.jit
def pallas_standalone__gqa_block_cached__near_ridge_kernel(
    x: jax.Array,
    k_cache: jax.Array,
    v_cache: jax.Array,
    wq: jax.Array,
    wo: jax.Array,
):
    assert x.shape == (_B, _SQ, _D) and k_cache.shape == (_B, _HKV, _SK, _DH)
    hbm = pl.BlockSpec(memory_space=pltpu.HBM)
    bf16 = jnp.bfloat16
    return pl.pallas_call(
        _kernel,
        in_specs=[hbm] * 5,
        out_specs=hbm,
        out_shape=jax.ShapeDtypeStruct((_B, _SQ, _D), x.dtype),
        scratch_shapes=[
            pltpu.VMEM((_B, _SQ, _D), bf16),
            pltpu.VMEM((_HKV, _D, 512), bf16),
            pltpu.VMEM((_HKV, _D, 512), bf16),
            pltpu.VMEM((_NB, _SK, _DH), bf16),
            pltpu.VMEM((_NB, _SK, _DH), bf16),
            pltpu.VMEM((_M, _DH), bf16),
            pltpu.VMEM((_M, _SK), jnp.float32),
            pltpu.VMEM((_M, _SK), bf16),
            pltpu.VMEM((_M, 128), jnp.float32),
            pltpu.VMEM((_B, _SQ, _D), jnp.float32),
            pltpu.VMEM((_B, _SQ, _D), bf16),
            pltpu.SemaphoreType.DMA((_B,)),
            pltpu.SemaphoreType.DMA((_HKV,)),
            pltpu.SemaphoreType.DMA((_HKV,)),
            pltpu.SemaphoreType.DMA((_NB,)),
            pltpu.SemaphoreType.DMA((_NB,)),
            pltpu.SemaphoreType.DMA((_B,)),
        ],
        compiler_params=pltpu.CompilerParams(
            vmem_limit_bytes=100 * 1024 * 1024, disable_bounds_checks=True),
    )(x, wq, wo.T, k_cache, v_cache)
```
